```python
import os as _os
_os.environ.setdefault("JAX_PLATFORMS", "cpu")
import jax
import jax.numpy as jnp

def _softmax(x, axis=-1):
    return jax.nn.softmax(x, axis=axis)
def _gelu(x):
    return jax.nn.gelu(x, approximate=True)
def _silu(x):
    return jax.nn.silu(x)
def _sigmoid(x):
    return jax.nn.sigmoid(x)
def _layernorm(x, axis=-1, eps=1e-5):
    m = jnp.mean(x, axis=axis, keepdims=True)
    v = jnp.var(x, axis=axis, keepdims=True)
    return (x - m) / jnp.sqrt(v + eps)
def _scatter_add(tgt, idx, src, axis=0):
    return tgt.at[idx].add(src)
def _segment_sum(src, seg, n):
    return jax.ops.segment_sum(src, seg, n)
class _Rng:
    def __init__(self, key):
        self._k = key
    def _next(self):
        self._k, sub = jax.random.split(self._k)
        return sub
    def normal(self, shape):
        return jax.random.normal(self._next(), shape, dtype=jnp.bfloat16)
    def randint(self, lo, hi, shape):
        return jax.random.randint(self._next(), shape, lo, hi, dtype=jnp.int32)
    def uniform(self, shape, lo=0.0, hi=1.0):
        return jax.random.uniform(self._next(), shape, jnp.bfloat16, lo, hi)
    def permutation(self, n):
        return jax.random.permutation(self._next(), n)


kernel_name = 'gated_mix__sliding_local_dilated__moe_arch_mod__prompt'

def setup_inputs():
    _rng = _Rng(jax.random.key(int.from_bytes(__import__("os").urandom(4), "little")))
    _w = (lambda a: (lambda t: t.astype(jnp.bfloat16) if jnp.issubdtype(t.dtype, jnp.floating) else t)(jnp.asarray(a)))
    def _A_setup():
        B, S, D = 1, 2048, 640
        return {
            "x": _w((lambda *s: _rng.normal(s) * 0.05)(B, S, D)),
            "wqkv": _w((lambda *s: _rng.normal(s) * 0.8)(D, 3 * D)),
            "wo": _w((lambda *s: _rng.normal(s) * 0.05)(D, D)),
        }
    _A_in = _A_setup()

    def _B_setup():
        B, S, D, F, C = 1, 2048, 640, 1728, 1
        return {
            "x": _w((lambda *s: _rng.normal(s) * 0.05)(B, S, D)),
            "w_r": _w((lambda *s: _rng.normal(s) * 1.6)(D)),
            "w_gate": _w((lambda *s: _rng.normal(s) * 0.4)(D, F)),
            "w_up": _w((lambda *s: _rng.normal(s) * 0.4)(D, F)),
            "w_down": _w((lambda *s: _rng.normal(s) * 0.4)(F, D)),
        }
    _B_in = _B_setup()

    return {
        "A_x": _A_in["x"],
        "A_wqkv": _A_in["wqkv"],
        "A_wo": _A_in["wo"],
        "B_x": _B_in["x"],
        "B_w_r": _B_in["w_r"],
        "B_w_gate": _B_in["w_gate"],
        "B_w_up": _B_in["w_up"],
        "B_w_down": _B_in["w_down"],
        "gate_w": _w((lambda *s: _rng.normal(s) * 0.05)(640) * 16.0),
    }

def reference(A_x, A_wqkv, A_wo, B_x, B_w_r, B_w_gate, B_w_up, B_w_down, gate_w):
    def _A_ref(x, wqkv, wo):
        B, S, D = x.shape
        H = 32; Dh = D // H
        W, dil = 8, 2
        qkv = (lambda x, *d: x.transpose(*d))((x @ wqkv).reshape(B, S, 3, H, Dh), 2, 0, 3, 1, 4)
        q, k, v = qkv[0], qkv[1], qkv[2]
        scale = Dh ** -0.5
        pos = jnp.arange(S)
        off = jnp.arange(W) * dil
        idx = pos[:, None] - off[None, :]
        mask = idx >= 0
        idx_c = jnp.where(mask, idx, 0).reshape(-1)
        kg = k[:, :, idx_c, :].reshape(B, H, S, W, Dh)
        vg = v[:, :, idx_c, :].reshape(B, H, S, W, Dh)
        logits = jnp.einsum("bhsd,bhswd->bhsw", q, kg) * scale
        logits = jnp.where(mask[None, None, :, :], logits, -1e9)
        attn = _softmax(logits, axis=-1)
        o = jnp.einsum("bhsw,bhswd->bhsd", attn, vg)
        return (lambda x, *d: x.transpose(*d))(o, 0, 2, 1, 3).reshape(B, S, D) @ wo

    def _B_ref(x, w_r, w_gate, w_up, w_down):
        B, S, D = x.shape
        C = 1
        r = x @ w_r
        idx = jnp.argsort(-r, axis=-1)[:, :C]
        idx_e = jnp.repeat(idx.reshape(B, C, 1), D, axis=2)
        x_sel = jnp.take_along_axis(x, idx_e, axis=1)
        g = _silu(x_sel @ w_gate)
        u = x_sel @ w_up
        y = (g * u) @ w_down
        r_sel = _sigmoid(jnp.take_along_axis(r, idx, axis=1))
        y = y * r_sel.reshape(B, C, 1)
        b_off = (jnp.arange(B) * S).reshape(B, 1)
        flat_idx = (idx + b_off).reshape(B * C)
        zero = (x * 0.0).reshape(B * S, D)
        upd = _scatter_add(zero, flat_idx, y.reshape(B * C, D), axis=0)
        return x + upd.reshape(B, S, D)

    x = A_x
    g = _sigmoid((x * gate_w).sum(-1, keepdims=True))
    a = _A_ref(x, A_wqkv, A_wo)
    b = _B_ref(x, B_w_r, B_w_gate, B_w_up, B_w_down)
    return g * a + (1 - g) * b
```

```python
import jax
import jax.numpy as jnp
import jax.experimental.pallas as pl
import jax.experimental.pallas.tpu as pltpu

S = 2048
D = 640
H = 32
DH = 20
WIN = 8
DIL = 2
F = 1728
NL = D // 128
HALO = 16
CH = 64
NCK = S // CH
T0 = 256
RG = 8
XR_AT = 8
FFN_AT = 16
YCH = 28
FR = 16
NSPLIT = 9
NGATE = 3
OT = 256
X1 = XR_AT * CH
NOP = S // OT - 2 + 2 * OT // CH
LOG2E = 1.4426950408889634
QSCALE = DH ** -0.5 * LOG2E
NEG = -1e9 * LOG2E
NT = (((1,), (1,)), ((), ()))
f32 = jnp.float32
bf16 = jnp.bfloat16
u32 = jnp.uint32


def _pk(v):
    return pltpu.bitcast(v, u32)


def _upk(v):
    return pltpu.bitcast(v, bf16)


def _sigmoid(z):
    return 0.5 * jnp.tanh(0.5 * z) + 0.5


def _kernel(z_ref, x_hbm, w_hbm, wo_hbm, wg_hbm, wu_hbm, wd_hbm, wr_ref, gw_ref, o_hbm,
            xv, wraw, wtp, t_scr, woraw, wof, wop, wg, wu, wd,
            q_s, k_s, v_s, l_s, o_s, a_s, gr_s, ov, xs_s, yacc_s, sel_s, acc_s,
            sem_w, sem_x, sem_m, sem_o):
    cw = [pltpu.make_async_copy(w_hbm.at[pl.ds(kk * 128, 128)], wraw.at[pl.ds(kk * 128, 128)], sem_w.at[kk])
          for kk in range(NL)]
    cwo = pltpu.make_async_copy(wo_hbm, woraw, sem_w.at[NL])
    cx0 = pltpu.make_async_copy(x_hbm.at[pl.ds(0, T0)], xv.at[pl.ds(0, T0)], sem_x.at[0])
    cx1 = pltpu.make_async_copy(x_hbm.at[pl.ds(T0, X1 - T0)], xv.at[pl.ds(T0, X1 - T0)], sem_x.at[1])
    cxr = pltpu.make_async_copy(x_hbm.at[pl.ds(X1, S - X1)], xv.at[pl.ds(X1, S - X1)], sem_x.at[2])
    cm = [pltpu.make_async_copy(wg_hbm, wg, sem_m.at[0]),
          pltpu.make_async_copy(wu_hbm, wu, sem_m.at[1]),
          pltpu.make_async_copy(wd_hbm, wd, sem_m.at[2])]
    opieces = [(t * OT, OT) for t in range(S // OT - 2)] + [(S - 2 * OT + c * CH, CH) for c in range(2 * OT // CH)]
    co = [pltpu.make_async_copy(ov.at[pl.ds(r0, n)], o_hbm.at[pl.ds(r0, n)], sem_o.at[i])
          for i, (r0, n) in enumerate(opieces)]

    cw[0].start()
    cx0.start()
    cw[1].start()

    for j in range(NL):
        k_s[j, 0:HALO, :] = jnp.zeros((HALO, 128), f32)
        v_s[j, 0:HALO, :] = jnp.zeros((HALO, 128), f32)
    ov[S:S + 16, :] = jnp.zeros((16, D), bf16)
    gr_s[2 * CH:2 * CH + 8, :] = jnp.zeros((8, 128), f32)
    l_s[0, S:S + 8, :] = jnp.zeros((8, 128), f32)

    yacc_s[FR:FR + 8, 0:128] = jnp.zeros((8, 128), f32)
    yacc = yacc_s.at[pl.ds(0, FR)]

    def permute_w_part(kk, t):
        for c in range(t * NL, (t + 1) * NL):
            blk = wraw[kk * 128:(kk + 1) * 128, c * 128:(c + 1) * 128].astype(f32)
            t_scr[kk % 2, c * 128:(c + 1) * 128, :] = blk.T
        for d in range(DH):
            rows = t_scr[kk % 2, pl.ds(t * D + d, H, stride=DH), :]
            n0 = (t * D + d * H) // 2
            wtp[n0:n0 + H // 2, kk * 128:(kk + 1) * 128] = _pk(rows.astype(bf16))

    def permute_wo():
        for j in range(NL):
            wof[j, :, :] = woraw[:, j * 128:(j + 1) * 128].astype(f32)
        for d in range(DH):
            for j in range(NL):
                rows = wof[j, pl.ds(d, H, stride=DH), :]
                wop[d * H // 2:(d + 1) * H // 2, j * 128:(j + 1) * 128] = _pk(rows.astype(bf16))

    def store_qkv(r, r0, nrows, n0, n1):
        for n in range(n0, n1):
            blk = r[:, (n - n0) * 128:(n - n0 + 1) * 128]
            if n < NL:
                q_s[n, r0:r0 + nrows, :] = blk * QSCALE
            elif n < 2 * NL:
                k_s[n - NL, HALO + r0:HALO + r0 + nrows, :] = blk
            else:
                v_s[n - 2 * NL, HALO + r0:HALO + r0 + nrows, :] = blk

    def pin_zero():
        z = z_ref[0]
        a = ov[pl.ds(pl.multiple_of(z + S, 16), 16), 0:128].astype(f32)
        b = gr_s[pl.ds(pl.multiple_of(z + 2 * CH, 8), 8), :]
        c = yacc_s[pl.ds(pl.multiple_of(z + FR, 8), 8), 0:128]
        return (a[0:8] + b) + c

    def qkv_rows(r0, nrows, n0, n1, pin):
        lhs = xv[r0:r0 + nrows, :]
        if pin:
            zero = l_s[0, pl.ds(pl.multiple_of(z_ref[0] + S, 8), 8), :]
            zero = pltpu.bitcast(zero + pin_zero(), u32)
            lhs = _upk(_pk(lhs) | jnp.tile(zero, (nrows // 16, NL)))
        r = jax.lax.dot_general(lhs, _upk(wtp[n0 * 64:n1 * 64, :]), NT, preferred_element_type=f32)
        store_qkv(r, r0, nrows, n0, n1)

    def qk_unit(r0):
        q = [q_s[j, r0:r0 + RG, :] for j in range(NL)]
        for w in range(WIN):
            o = HALO + r0 - DIL * w
            s = q[0] * k_s[0, o:o + RG, :]
            for j in range(1, NL):
                s = s + q[j] * k_s[j, o:o + RG, :]
            l_s[w, r0:r0 + RG, :] = (s + pltpu.roll(s, 64, 1)) + (pltpu.roll(s, 32, 1) + pltpu.roll(s, 96, 1))

    def pv_unit(r0):
        ls = [l_s[w, r0:r0 + RG, :] for w in range(WIN)]
        if r0 < DIL * (WIN - 1):
            pos = r0 + jax.lax.broadcasted_iota(jnp.int32, (RG, 128), 0)
            ls = [ls[0]] + [jnp.where(pos >= DIL * w, ls[w], NEG) for w in range(1, WIN)]
        m = jnp.maximum(jnp.maximum(jnp.maximum(ls[0], ls[1]), jnp.maximum(ls[2], ls[3])),
                        jnp.maximum(jnp.maximum(ls[4], ls[5]), jnp.maximum(ls[6], ls[7])))
        ps = [jnp.exp2(l - m) for l in ls]
        den = ((ps[0] + ps[1]) + (ps[2] + ps[3])) + ((ps[4] + ps[5]) + (ps[6] + ps[7]))
        inv = pl.reciprocal(den, approx=True)
        inv = inv * (2.0 - den * inv)
        for j in range(NL):
            acc = None
            for w in range(WIN):
                o = HALO + r0 - DIL * w
                t = ps[w] * v_s[j, o:o + RG, :]
                acc = t if acc is None else acc + t
            o_s[r0 // 2:(r0 + RG) // 2, j * 128:(j + 1) * 128] = _pk((acc * inv).astype(bf16))

    def qk_chunk(i):
        for g in range(CH // RG):
            qk_unit(i * CH + g * RG)

    def pv_chunk(i):
        for g in range(CH // RG):
            pv_unit(i * CH + g * RG)

    def wo_chunk(i):
        r0 = i * CH
        a_s[r0:r0 + CH, :] = jnp.dot(_upk(o_s[r0 // 2:(r0 + CH) // 2, :]), _upk(wop[...]),
                                     preferred_element_type=f32)

    def router(i):
        r0 = i * CH
        pr = None
        for j in range(NL):
            b = xv[r0:r0 + CH, j * 128:(j + 1) * 128].astype(f32) * wr_ref[j:j + 1, :].astype(f32)
            pr = b if pr is None else pr + b
        r = jnp.sum(pr, axis=1, keepdims=True).astype(bf16).astype(f32)
        pos = (r0 + jax.lax.broadcasted_iota(jnp.int32, (CH, 1), 0)).astype(f32)
        if i == 0:
            gr_s[0:CH, 0:1] = r
            gr_s[CH:2 * CH, 0:1] = pos
        else:
            m = gr_s[0:CH, 0:1]
            better = r > m
            gr_s[0:CH, 0:1] = jnp.where(better, r, m)
            gr_s[CH:2 * CH, 0:1] = jnp.where(better, pos, gr_s[CH:2 * CH, 0:1])

    def final_rows(rows, n, pos0, with_y, drows=None):
        drows = rows if drows is None else drows
        xf = [xv[rows, j * 128:(j + 1) * 128].astype(f32) for j in range(NL)]
        pg = None
        for j in range(NL):
            a = xf[j] * gw_ref[j:j + 1, :].astype(f32)
            pg = a if pg is None else pg + a
        g = jnp.broadcast_to(_sigmoid(jnp.sum(pg, axis=1, keepdims=True)), (n, 128))
        g1 = 1.0 - g
        if with_y:
            pos = (pos0 + jax.lax.broadcasted_iota(jnp.int32, (n, 128), 0)).astype(f32)
            hit = pos == sel_s[0:1, 0:128]
        for j in range(NL):
            cs = slice(j * 128, (j + 1) * 128)
            b = xf[j]
            if with_y:
                b = b + jnp.where(hit, sel_s[8:9, cs], 0.0)
            ov[drows, cs] = (g * a_s[rows, cs] + g1 * b).astype(bf16)

    st = {}

    def moe_select():
        r = gr_s[0:CH, 0:1]
        rmax = jnp.max(r, axis=0, keepdims=True)
        idx = jnp.min(jnp.where(r == rmax, gr_s[CH:2 * CH, 0:1], S - 1.0), axis=0, keepdims=True)
        idx_s = idx.astype(jnp.int32)[0, 0]
        st['idx'] = idx_s
        base = pl.multiple_of((idx_s // 16) * 16, 16)
        x16 = xv[pl.ds(base, 16), :]
        row = base + jax.lax.broadcasted_iota(jnp.int32, (16, D), 0)
        xsel = jnp.where(row == idx_s, x16.astype(f32), 0.0)
        xsel = jnp.sum(xsel, axis=0, keepdims=True)
        xs_s[...] = jnp.broadcast_to(xsel, (FR, D))
        sel_s[0:8, :] = jnp.broadcast_to(idx, (8, D))
        sel_s[16:24, :] = jnp.broadcast_to(_sigmoid(rmax), (8, D))

    FB = [(f0, min(f0 + 128, F)) for f0 in range(0, F, 128)]

    def moe_piece(p):
        f0, f1 = FB[p]
        xs = [xs_s[:, j * 128:(j + 1) * 128] for j in range(NL)]
        y = None if p == 0 else [yacc[:, j * 128:(j + 1) * 128] for j in range(NL)]
        for r in range(f0, f1, FR):
            ag = au = None
            for j in range(NL):
                cs = slice(j * 128, (j + 1) * 128)
                a = wg[r:r + FR, cs].astype(f32) * xs[j]
                b = wu[r:r + FR, cs].astype(f32) * xs[j]
                ag = a if ag is None else ag + a
                au = b if au is None else au + b
            hg = jnp.sum(ag, axis=1, keepdims=True)
            hu = jnp.sum(au, axis=1, keepdims=True)
            h = jnp.broadcast_to((hg * _sigmoid(hg)) * hu, (FR, 128))
            t = [h * wd[r:r + FR, j * 128:(j + 1) * 128].astype(f32) for j in range(NL)]
            y = t if y is None else [y[j] + t[j] for j in range(NL)]
        for j in range(NL):
            yacc[:, j * 128:(j + 1) * 128] = y[j]
        if p == len(FB) - 1:
            ysum = jnp.sum(yacc[...], axis=0, keepdims=True)
            sel_s[8:16, :] = jnp.broadcast_to(ysum, (8, D)) * sel_s[16:24, :]

    for kk in range(NL + 1):
        if kk < NL:
            cw[kk].wait()
            if kk == 0:
                cw[2].start()
            elif kk == 1:
                cx0.wait()
                cw[3].start()
            elif kk == 2:
                cw[4].start()
            elif kk == 3:
                cwo.start()
                cx1.start()
            elif kk == 4:
                cxr.start()
            for t in range(3):
                permute_w_part(kk, t)
        if kk >= 1:
            ks = slice((kk - 1) * 128, kk * 128)
            p = jax.lax.dot_general(xv[0:T0, ks], _upk(wtp[:, ks]), NT, preferred_element_type=f32)
            if kk == 1:
                acc_s[...] = p
            elif kk < NL:
                acc_s[...] = acc_s[...] + p
            else:
                store_qkv(acc_s[...] + p, 0, T0, 0, 3 * NL)

    nq0 = T0 // CH
    routers_todo = list(range(NCK))
    finals_todo = []
    fin_done = [False] * NCK
    started = []
    ctl = {'y': False}

    def emit_finals(n):
        for _ in range(n):
            if not finals_todo or (finals_todo[0] >= YCH and not ctl['y']):
                break
            i = finals_todo.pop(0)
            final_rows(slice(i * CH, (i + 1) * CH), CH, i * CH, i >= YCH)
            fin_done[i] = True
            for pi, (r0, nr) in enumerate(opieces):
                if pi not in started and all(fin_done[c] for c in range(r0 // CH, (r0 + nr) // CH)):
                    co[pi].start()
                    started.append(pi)

    def patch_compute():
        base = pl.multiple_of((jnp.minimum(st['idx'], YCH * CH - 1) // 16) * 16, 16)
        final_rows(pl.ds(base, 16), 16, base, True, slice(S + 16, S + 32))
        st['patch'] = pltpu.make_async_copy(ov.at[pl.ds(S + 16, 16)], o_hbm.at[pl.ds(base, 16)], sem_o.at[NOP])

    def side_work(q):
        xlim = XR_AT if q < XR_AT else NCK
        for _ in range(NGATE):
            if routers_todo and routers_todo[0] < xlim:
                router(routers_todo.pop(0))
        emit_finals(2)
        k = q - FFN_AT
        if 0 <= k < len(FB):
            moe_piece(k)
            ctl['y'] = k == len(FB) - 1
        if q == NCK - 1:
            patch_compute()

    def finish(i):
        pv_chunk(i)
        wo_chunk(i)
        finals_todo.append(i)

    next_attn = 0
    for q in range(nq0, NCK):
        if q == nq0:
            cwo.wait()
            cx1.wait()
            for c in cm:
                c.start()
            permute_wo()
        elif q == XR_AT:
            cxr.wait()
        elif q == FFN_AT:
            for c in cm:
                c.wait()
        todo = list(range(next_attn, min(q, next_attn + 2)))
        if len(todo) == 2:
            a, b = todo
            qkv_rows(q * CH, CH, 0, 5, False)
            qk_chunk(a)
            side_work(q)
            qkv_rows(q * CH, CH, 5, 10, True)
            finish(a)
            qk_chunk(b)
            qkv_rows(q * CH, CH, 10, 15, True)
            finish(b)
        else:
            qkv_rows(q * CH, CH, 0, NSPLIT, False)
            qk_chunk(todo[0])
            side_work(q)
            qkv_rows(q * CH, CH, NSPLIT, 3 * NL, True)
            finish(todo[0])
        if q == FFN_AT - 1:
            assert not routers_todo
            moe_select()
        next_attn += len(todo)
    while next_attn < NCK:
        emit_finals(NCK)
        qk_chunk(next_attn)
        finish(next_attn)
        next_attn += 1
    emit_finals(NCK)
    assert len(started) == len(opieces)
    for pi, (r0, nr) in enumerate(opieces):
        if r0 + nr <= YCH * CH:
            co[pi].wait()
    st['patch'].start()
    for pi, (r0, nr) in enumerate(opieces):
        if r0 + nr > YCH * CH:
            co[pi].wait()
    st['patch'].wait()


@jax.jit
def pallas_gated_mix__sliding_local_dilated__moe_arch_mod__prompt_kernel(
    A_x: jax.Array,
    A_wqkv: jax.Array,
    A_wo: jax.Array,
    B_x: jax.Array,
    B_w_r: jax.Array,
    B_w_gate: jax.Array,
    B_w_up: jax.Array,
    B_w_down: jax.Array,
    gate_w: jax.Array,
):
    B = A_x.shape[0]
    x = A_x.reshape(S, D)
    any_spec = pl.BlockSpec(memory_space=pl.ANY)
    vmem_spec = pl.BlockSpec(memory_space=pltpu.VMEM)
    out = pl.pallas_call(
        _kernel,
        out_shape=jax.ShapeDtypeStruct((S, D), bf16),
        in_specs=[pl.BlockSpec(memory_space=pltpu.SMEM)] + [any_spec] * 6 + [vmem_spec] * 2,
        out_specs=any_spec,
        scratch_shapes=[
            pltpu.VMEM((S, D), bf16),
            pltpu.VMEM((D, 3 * D), bf16),
            pltpu.VMEM((3 * D // 2, D), u32),
            pltpu.VMEM((2, 3 * D, 128), f32),
            pltpu.VMEM((D, D), bf16),
            pltpu.VMEM((NL, D, 128), f32),
            pltpu.VMEM((D // 2, D), u32),
            pltpu.VMEM((F, D), bf16),
            pltpu.VMEM((F, D), bf16),
            pltpu.VMEM((F, D), bf16),
            pltpu.VMEM((NL, S, 128), f32),
            pltpu.VMEM((NL, S + HALO, 128), f32),
            pltpu.VMEM((NL, S + HALO, 128), f32),
            pltpu.VMEM((WIN, S + 8, 128), f32),
            pltpu.VMEM((S // 2, D), u32),
            pltpu.VMEM((S, D), f32),
            pltpu.VMEM((2 * CH + 8, 128), f32),
            pltpu.VMEM((S + 32, D), bf16),
            pltpu.VMEM((FR, D), f32),
            pltpu.VMEM((FR + 8, D), f32),
            pltpu.VMEM((24, D), f32),
            pltpu.VMEM((T0, 3 * D), f32),
            pltpu.SemaphoreType.DMA((NL + 1,)),
            pltpu.SemaphoreType.DMA((3,)),
            pltpu.SemaphoreType.DMA((3,)),
            pltpu.SemaphoreType.DMA((NOP + 1,)),
        ],
        compiler_params=pltpu.CompilerParams(vmem_limit_bytes=110 * 1024 * 1024),
    )(jnp.zeros((1,), jnp.int32), x, A_wqkv, A_wo, B_w_gate.T, B_w_up.T, B_w_down,
      B_w_r.reshape(NL, 128), gate_w.reshape(NL, 128))
    return out.reshape(B, S, D)
```
